```python
import os as _os
_os.environ.setdefault("JAX_PLATFORMS", "cpu")
import jax
import jax.numpy as jnp

def _softmax(x, axis=-1):
    return jax.nn.softmax(x, axis=axis)
def _gelu(x):
    return jax.nn.gelu(x, approximate=True)
def _silu(x):
    return jax.nn.silu(x)
def _sigmoid(x):
    return jax.nn.sigmoid(x)
def _layernorm(x, axis=-1, eps=1e-5):
    m = jnp.mean(x, axis=axis, keepdims=True)
    v = jnp.var(x, axis=axis, keepdims=True)
    return (x - m) / jnp.sqrt(v + eps)
def _scatter_add(tgt, idx, src, axis=0):
    return tgt.at[idx].add(src)
def _segment_sum(src, seg, n):
    return jax.ops.segment_sum(src, seg, n)
class _Rng:
    def __init__(self, key):
        self._k = key
    def _next(self):
        self._k, sub = jax.random.split(self._k)
        return sub
    def normal(self, shape):
        return jax.random.normal(self._next(), shape, dtype=jnp.bfloat16)
    def randint(self, lo, hi, shape):
        return jax.random.randint(self._next(), shape, lo, hi, dtype=jnp.int32)
    def uniform(self, shape, lo=0.0, hi=1.0):
        return jax.random.uniform(self._next(), shape, jnp.bfloat16, lo, hi)
    def permutation(self, n):
        return jax.random.permutation(self._next(), n)


kernel_name = 'concat_heads__sliding_local_dilated__compressed_kv_cla__prompt'

def setup_inputs():
    _rng = _Rng(jax.random.key(int.from_bytes(__import__("os").urandom(4), "little")))
    _w = (lambda a: (lambda t: t.astype(jnp.bfloat16) if jnp.issubdtype(t.dtype, jnp.floating) else t)(jnp.asarray(a)))
    def _A_setup():
        B, S, D = 1, 2048, 640
        return {
            "x": _w((lambda *s: _rng.normal(s) * 0.2)(B, S, D)),
            "wqkv": _w((lambda *s: _rng.normal(s) * 0.2)(D, 3 * D)),
            "wo": _w((lambda *s: _rng.normal(s) * 0.05)(D, D)),
        }
    _A_in = _A_setup()

    def _B_setup():
        B, H, Sq, Sk, D, M = 1, 32, 2048, 2048, 128, 640
        Dc = 4 * D
        return {
            "x": _w((lambda *s: _rng.normal(s) * 0.8)(B, Sq, M)),
            "c_kv": _w((lambda *s: _rng.normal(s) * 0.8)(B, Sk, Dc)),
            "w_q": _w((lambda *s: _rng.normal(s) * 1.6)(M, H, D) * (M ** -0.5)),
            "w_uk": _w((lambda *s: _rng.normal(s) * 1.6)(Dc, H, D) * (Dc ** -0.5)),
            "w_uv": _w((lambda *s: _rng.normal(s) * 0.8)(Dc, H, D) * (Dc ** -0.5)),
            "w_o": _w((lambda *s: _rng.normal(s) * 0.8)(H, D, M) * ((H * D) ** -0.5)),
        }
    _B_in = _B_setup()

    return {
        "A_x": _A_in["x"],
        "A_wqkv": _A_in["wqkv"],
        "A_wo": _A_in["wo"],
        "B_x": _B_in["x"],
        "B_c_kv": _B_in["c_kv"],
        "B_w_q": _B_in["w_q"],
        "B_w_uk": _B_in["w_uk"],
        "B_w_uv": _B_in["w_uv"],
        "B_w_o": _B_in["w_o"],
    }

def reference(A_x, A_wqkv, A_wo, B_x, B_c_kv, B_w_q, B_w_uk, B_w_uv, B_w_o):
    def _A_ref(x, wqkv, wo):
        B, S, D = x.shape
        H = 32; Dh = D // H
        W, dil = 8, 2
        qkv = (lambda x, *d: x.transpose(*d))((x @ wqkv).reshape(B, S, 3, H, Dh), 2, 0, 3, 1, 4)
        q, k, v = qkv[0], qkv[1], qkv[2]
        scale = Dh ** -0.5
        pos = jnp.arange(S)
        off = jnp.arange(W) * dil
        idx = pos[:, None] - off[None, :]
        mask = idx >= 0
        idx_c = jnp.where(mask, idx, 0).reshape(-1)
        kg = k[:, :, idx_c, :].reshape(B, H, S, W, Dh)
        vg = v[:, :, idx_c, :].reshape(B, H, S, W, Dh)
        logits = jnp.einsum("bhsd,bhswd->bhsw", q, kg) * scale
        logits = jnp.where(mask[None, None, :, :], logits, -1e9)
        attn = _softmax(logits, axis=-1)
        o = jnp.einsum("bhsw,bhswd->bhsd", attn, vg)
        return (lambda x, *d: x.transpose(*d))(o, 0, 2, 1, 3).reshape(B, S, D) @ wo

    def _B_ref(x, c_kv, w_q, w_uk, w_uv, w_o):
        B, Sq, M = x.shape[0], x.shape[1], x.shape[2]
        Sk = c_kv.shape[1]
        H, D = w_q.shape[1], w_q.shape[2]
        q = jnp.einsum("bqm,mhd->bhqd", x, w_q)
        k = jnp.einsum("bkc,chd->bhkd", c_kv, w_uk)
        v = jnp.einsum("bkc,chd->bhkd", c_kv, w_uv)
        scores = jnp.einsum("bhqd,bhkd->bhqk", q, k) * (D ** -0.5)
        off = Sk - Sq
        qi = jnp.arange(Sq)[:, None]
        kj = jnp.arange(Sk)[None, :]
        cmask = kj <= (qi + off)
        scores = jnp.where(cmask[None, None], scores, -1e9)
        p = _softmax(scores, axis=-1)
        ctx = jnp.einsum("bhqk,bhkd->bhqd", p, v)
        return jnp.einsum("bhqd,hdm->bqm", ctx, w_o)

    a = _A_ref(A_x, A_wqkv, A_wo)
    b = _B_ref(B_x, B_c_kv, B_w_q, B_w_uk, B_w_uv, B_w_o)
    return jnp.concatenate([a, b], axis=-1)
```

```python
import functools

import numpy as np
import jax
import jax.numpy as jnp
import jax.experimental.pallas as pl
import jax.experimental.pallas.tpu as pltpu

_LOG2E = 1.4426950408889634
_NEG = -1e9

_A_HEADS = 32
_A_WIN = 8
_A_DIL = 2
_NSHIFT = 8 // _A_DIL
_HALO = 8

_BQ = 512
_SB = 128
_CA = 16
_RP = 512
_PJ = 1024
_RA = 512

_DBG = 0
_NT = (((1,), (1,)), ((), ()))


def _dot(a, b):
    return jnp.dot(a, b, preferred_element_type=jnp.float32)


def _recip(x):
    r = pl.reciprocal(x, approx=True)
    return r * (2.0 - x * r)


def _permute_wqkv(wqkv_ref, j, rows):
    D = wqkv_ref.shape[0]
    dh = D // _A_HEADS
    tiles = [pltpu.bitcast(wqkv_ref[rows, pl.ds(j * D + t, 128)], jnp.uint32) for t in range(0, D, 128)]
    lane = jax.lax.broadcasted_iota(jnp.int32, tiles[0].shape, 1)
    for t in range(0, D, 128):
        src = (lane % _A_HEADS) * dh + (lane + t) // _A_HEADS
        out = None
        for n, tile in enumerate(tiles):
            g = jnp.take_along_axis(tile, src % 128, axis=1)
            out = g if out is None else jnp.where(src // 128 == n, g, out)
        wqkv_ref[rows, pl.ds(j * D + t, 128)] = pltpu.bitcast(out, jnp.bfloat16)


def _permute_wo(wo_ref, out_ref):
    ntiles, D, _ = wo_ref.shape
    half = D // _A_HEADS // 2
    for t in range(ntiles):
        w32 = wo_ref.at[t].bitcast(jnp.uint32)
        for i in range(half):
            for k, rows in enumerate(_unpack_rows(w32[pl.ds(i, _A_HEADS, stride=half), :])):
                out_ref[pl.ds((2 * i + k) * _A_HEADS, _A_HEADS), pl.ds(t * 128, 128)] = rows


def _unpack_rows(w32):
    even = pltpu.bitcast(w32 << 16, jnp.float32).astype(jnp.bfloat16)
    odd = pltpu.bitcast(w32 & jnp.uint32(0xFFFF0000), jnp.float32).astype(jnp.bfloat16)
    return even, odd


def _project_a(j, r0, ax_ref, wqkv_ref, scr):
    D = ax_ref.shape[1]
    y = _dot(ax_ref[pl.ds(r0, _RP), :], wqkv_ref[:, j * D:(j + 1) * D])
    if j == 0:
        scr[pl.ds(r0, _RP), :] = y * ((D // _A_HEADS) ** -0.5 * _LOG2E)
    else:
        for n in range(_NSHIFT):
            scr.at[n, pl.ds(r0, _RP + 2 * _HALO), :][pl.ds(_HALO + n * _A_DIL, _RP), :] = y


def _attend_a(r0, wo_ref, o_ref, q_scr, k_scr, v_scr):
    D = wo_ref.shape[0]
    outs = []
    for c0 in range(r0, r0 + _RA, _CA):
        q = q_scr[c0:c0 + _CA, :]
        tap = lambda scr, w: scr[w % _NSHIFT, pl.ds(c0 + _HALO - w // _NSHIFT * 8, _CA), :]
        logits = []
        for w in range(_A_WIN):
            prod = q * tap(k_scr, w)
            lg = functools.reduce(jnp.add, [prod[:, t:t + 128] for t in range(0, D, 128)])
            lg = lg + pltpu.roll(lg, 2 * _A_HEADS, 1)
            lg = lg + pltpu.roll(lg, _A_HEADS, 1)
            if c0 < w * _A_DIL:
                pos = c0 + jax.lax.broadcasted_iota(jnp.int32, lg.shape, 0)
                lg = jnp.where(pos >= w * _A_DIL, lg, _NEG * _LOG2E)
            logits.append(lg)
        m = functools.reduce(jnp.maximum, logits)
        e = [jnp.exp2(lg - m) for lg in logits]
        inv = _recip(functools.reduce(jnp.add, e))
        o = None
        for w in range(_A_WIN):
            t = jnp.concatenate([e[w] * inv] * (D // 128), axis=1) * tap(v_scr, w)
            o = t if o is None else o + t
        outs.append(o.astype(jnp.bfloat16))
        if c0 + _CA < r0 + _RA:
            yield
    o = jnp.concatenate(outs, axis=0)
    o_ref[r0:r0 + _RA, 0:D] = _dot(o, wo_ref[...]).astype(o_ref.dtype)


def _head_pair(w32):
    return jnp.concatenate(_unpack_rows(w32), axis=1)


def _project(slot, rows, which, bx_ref, c_ref, wq_ref, wuk_ref, wuv_ref, q_scr, k_scr, v_scr):
    if which == 0:
        d = wq_ref.shape[2]
        q = _dot(bx_ref[rows, :], _head_pair(wq_ref[slot])) * (d ** -0.5 * _LOG2E)
        q_scr[slot, rows, :] = q.astype(jnp.bfloat16)
    else:
        c = c_ref[rows, :]
        k_scr[slot, :, rows] = _dot(c, _head_pair(wuk_ref[slot])).T.astype(jnp.bfloat16)
        v_scr[slot, rows, :] = _dot(c, _head_pair(wuv_ref[slot])).astype(jnp.bfloat16)


def _attend(pair, slot, hh, i, q_scr, k_scr, v_scr, ctx_scr):
    d = q_scr.shape[2] // 2
    hs = slice(hh * d, (hh + 1) * d)
    lo, hi = i * _BQ, (i + 1) * _BQ
    nsub = _BQ // _SB
    row = jax.lax.broadcasted_iota(jnp.int32, (_SB, _SB), 0)
    col = jax.lax.broadcasted_iota(jnp.int32, (_SB, _SB), 1)
    sub = lambda x, j: x[j * _SB:(j + 1) * _SB]
    q = q_scr[slot, lo:hi, hs]
    spans = ([(0, lo, 0)] if i > 0 else []) + [(lo + t * _SB, lo + (t + 1) * _SB, t) for t in range(nsub)]
    s = {}
    for n, (k0, k1, t) in enumerate(spans):
        sn = _dot(q[t * _SB:], k_scr[slot, hs, k0:k1])
        for j in range(t, nsub):
            sj = sub(sn, j - t)
            s[n, j] = jnp.where(col <= row, sj, _NEG * _LOG2E) if (k0 >= lo and j == t) else sj
    p, inv = {}, []
    for j in range(nsub):
        keys = [key for key in s if key[1] == j]
        tiles = [s[key][:, c:c + 128] for key in keys for c in range(0, s[key].shape[1], 128)]
        m = jnp.max(functools.reduce(jnp.maximum, tiles), axis=-1, keepdims=True)
        l = None
        for key in keys:
            cols = []
            for c in range(0, s[key].shape[1], 128):
                e = jnp.exp2(s[key][:, c:c + 128] - m)
                l = e if l is None else l + e
                cols.append(e.astype(jnp.bfloat16))
            p[key] = jnp.concatenate(cols, axis=1)
        inv.append(_recip(jnp.sum(l, axis=-1, keepdims=True)))
    ctx = [None] * nsub
    for n, (k0, k1, t) in enumerate(spans):
        pn = jnp.concatenate([p[n, j] for j in range(t, nsub)], axis=0)
        cn = _dot(pn, v_scr[slot, k0:k1, hs])
        for j in range(t, nsub):
            ctx[j] = sub(cn, j - t) if ctx[j] is None else ctx[j] + sub(cn, j - t)
    for j in range(nsub):
        ctx_scr[pair, lo + j * _SB:lo + (j + 1) * _SB, hs] = (ctx[j] * inv[j]).astype(jnp.bfloat16)


def _kernel(ax_hbm, wqkv_hbm, wo_hbm, bx_hbm, c_hbm, wq_hbm, wuk_hbm, wuv_hbm, wob_hbm, o_hbm,
            ax, wqkv, wo_raw, bx, c, wob, wo, ob, wq2, wuk2, wuv2,
            qa_scr, ka_scr, va_scr, q_scr, k_scr, v_scr, ctx_scr, in_sem, wa_sem, wo_sem, w_sem, ob_sem):
    S, DA = ax.shape
    M = bx.shape[1]
    npairs = ctx_scr.shape[0]
    srcs = (ax_hbm, bx_hbm, c_hbm, wob_hbm)
    dsts = (ax, bx, c, wob)
    loads = [pltpu.make_async_copy(s, t, in_sem.at[n]) for n, (s, t) in enumerate(zip(srcs, dsts))]

    wo_loads = [pltpu.make_async_copy(wo_hbm.at[:, pl.ds(t * 128, 128)], wo_raw.at[t], wo_sem.at[t])
                for t in range(DA // 128)]

    def pair_loads(pair):
        return [pltpu.make_async_copy(w.bitcast(jnp.uint32).at[:, pair, :], t.at[pair % 2], w_sem.at[n, pair % 2])
                for n, (w, t) in enumerate(((wq_hbm, wq2), (wuk_hbm, wuk2), (wuv_hbm, wuv2)))]

    wqkv_loads = [pltpu.make_async_copy(wqkv_hbm.at[:, pl.ds(j * DA, DA)], wqkv.at[:, pl.ds(j * DA, DA)],
                                        wa_sem.at[j]) for j in range(3)]
    for cp in (wqkv_loads[0], loads[0], wqkv_loads[1]):
        cp.start()
    ka_scr[:, 0:2 * _HALO, :] = jnp.zeros((_NSHIFT, 2 * _HALO, DA), jnp.float32)
    va_scr[:, 0:2 * _HALO, :] = jnp.zeros((_NSHIFT, 2 * _HALO, DA), jnp.float32)
    wqkv_loads[0].wait()
    _permute_wqkv(wqkv, 0, pl.ds(0, DA))
    loads[0].wait()
    for cp in wqkv_loads[2:] + wo_loads + loads[1:3] + pair_loads(0) + pair_loads(1) + loads[3:]:
        cp.start()
    nblk = S // _RP
    wrows = DA // nblk
    for j, scr in enumerate((qa_scr, ka_scr, va_scr)):
        if j < 2:
            wqkv_loads[j + 1].wait()

        @pl.loop(0, nblk)
        def _(blk):
            _project_a(j, pl.multiple_of(blk * _RP, _RP), ax, wqkv, scr)
            if j < 2:
                _permute_wqkv(wqkv, j + 1, pl.ds(pl.multiple_of(blk * wrows, wrows), wrows))

    for cp in wo_loads + loads[1:3] + pair_loads(0):
        cp.wait()

    proj = (bx, c, wq2, wuk2, wuv2, q_scr, k_scr, v_scr)
    qkv = (q_scr, k_scr, v_scr, ctx_scr)
    nq = S // _BQ
    _permute_wo(wo_raw, wo)
    for which in range(2):
        _project(0, slice(0, S), which, *proj)

    @pl.loop(0, npairs - 1)
    def _(pair):
        slot = pair % 2

        @pl.when(pair + 2 < npairs)
        def _():
            for cp in pair_loads(pair + 2):
                cp.start()

        for cp in pair_loads(pair + 1):
            cp.wait()
        for i in reversed(range(nq)):
            for hh in range(2):
                _attend(pair, slot, hh, i, *qkv)
                if (i * _BQ) % _PJ == 0:
                    _project(1 - slot, slice(i * _BQ, i * _BQ + _PJ), hh, *proj)

    loads[3].wait()
    stores_b = []
    for i in reversed(range(nq)):
        for hh in range(2):
            _attend(npairs - 1, (npairs - 1) % 2, hh, i, *qkv)
        rows = slice(i * _BQ, (i + 1) * _BQ)
        for r0 in range(i * _BQ, (i + 1) * _BQ, _RA):
            mixer_a = _attend_a(r0, wo, ob, qa_scr, ka_scr, va_scr)
            ctx = jnp.concatenate([ctx_scr[p, r0:r0 + _RA, :] for p in range(npairs)], axis=1)
            for n0 in range(0, M, 128):
                ob[r0:r0 + _RA, DA + n0:DA + n0 + 128] = _dot(ctx, wob[:, n0:n0 + 128]).astype(ob.dtype)
                for _ in range(_RA // _CA * 128 // M):
                    next(mixer_a)
            for _ in mixer_a:
                pass
        cp = pltpu.make_async_copy(ob.at[rows, :], o_hbm.at[rows, :], ob_sem.at[i])
        cp.start()
        stores_b.append(cp)
    for cp in stores_b:
        cp.wait()


@jax.jit
def pallas_concat_heads__sliding_local_dilated__compressed_kv_cla__prompt_kernel(
    A_x: jax.Array,
    A_wqkv: jax.Array,
    A_wo: jax.Array,
    B_x: jax.Array,
    B_c_kv: jax.Array,
    B_w_q: jax.Array,
    B_w_uk: jax.Array,
    B_w_uv: jax.Array,
    B_w_o: jax.Array,
):
    B, S, DA = A_x.shape
    _, _, M = B_x.shape
    _, Sk, Dc = B_c_kv.shape
    _, H, d = B_w_q.shape
    assert DA % 128 == 0 and 4 * _A_HEADS == 128 and B == 1 and Sk == S and H % 2 == 0
    bf16 = jnp.bfloat16
    operands = (A_x.reshape(S, DA), A_wqkv, A_wo, B_x.reshape(S, M), B_c_kv.reshape(Sk, Dc),
                B_w_q, B_w_uk, B_w_uv,
                B_w_o.reshape(H * d, M))
    assert all(a.dtype == bf16 for a in operands)
    hbm = pl.BlockSpec(memory_space=pltpu.HBM)
    out = pl.pallas_call(
        _kernel,
        in_specs=[hbm] * len(operands),
        out_specs=hbm,
        out_shape=jax.ShapeDtypeStruct((S, DA + M), bf16),
        scratch_shapes=[
            pltpu.VMEM((S, DA), bf16),
            pltpu.VMEM((DA, 3 * DA), bf16),
            pltpu.VMEM((DA // 128, DA, 128), bf16),
            pltpu.VMEM((S, M), bf16),
            pltpu.VMEM((Sk, Dc), bf16),
            pltpu.VMEM((H * d, M), bf16),
            pltpu.VMEM((DA, DA), bf16),
            pltpu.VMEM((S, DA + M), bf16),
            pltpu.VMEM((2, M, d), jnp.uint32),
            pltpu.VMEM((2, Dc, d), jnp.uint32),
            pltpu.VMEM((2, Dc, d), jnp.uint32),
            pltpu.VMEM((S, DA), jnp.float32),
            pltpu.VMEM((_NSHIFT, S + 2 * _HALO, DA), jnp.float32),
            pltpu.VMEM((_NSHIFT, S + 2 * _HALO, DA), jnp.float32),
            pltpu.VMEM((2, S, 2 * d), bf16),
            pltpu.VMEM((2, 2 * d, S), bf16),
            pltpu.VMEM((2, S, 2 * d), bf16),
            pltpu.VMEM((H // 2, S, 2 * d), bf16),
            pltpu.SemaphoreType.DMA((4,)),
            pltpu.SemaphoreType.DMA((3,)),
            pltpu.SemaphoreType.DMA((DA // 128,)),
            pltpu.SemaphoreType.DMA((3, 2)),
            pltpu.SemaphoreType.DMA((S // _BQ,)),
        ],
        compiler_params=pltpu.CompilerParams(vmem_limit_bytes=126 * 1024 * 1024),
    )(*operands)
    return out.reshape(B, S, DA + M)
```

```python
import functools

import jax
import jax.numpy as jnp
import jax.experimental.pallas as pl
import jax.experimental.pallas.tpu as pltpu

_LOG2E = 1.4426950408889634
_NEG = -1e9

_A_HEADS = 32
_A_WIN = 8
_A_DIL = 2
_NSHIFT = 8 // _A_DIL
_HALO = 8

_BQ = 512
_SB = 128
_CA = 16
_RP = 512
_RO = 256
_PJ = 1024


def _dot(a, b):
    return jnp.dot(a, b, preferred_element_type=jnp.float32)


def _recip(x):
    r = pl.reciprocal(x, approx=True)
    return r * (2.0 - x * r)


def _permute_wqkv(wqkv_ref, j, rows):
    D = wqkv_ref.shape[0]
    dh = D // _A_HEADS
    tiles = [pltpu.bitcast(wqkv_ref[rows, pl.ds(j * D + t, 128)], jnp.uint32) for t in range(0, D, 128)]
    lane = jax.lax.broadcasted_iota(jnp.int32, tiles[0].shape, 1)
    for t in range(0, D, 128):
        src = (lane % _A_HEADS) * dh + (lane + t) // _A_HEADS
        out = None
        for n, tile in enumerate(tiles):
            g = jnp.take_along_axis(tile, src % 128, axis=1)
            out = g if out is None else jnp.where(src // 128 == n, g, out)
        wqkv_ref[rows, pl.ds(j * D + t, 128)] = pltpu.bitcast(out, jnp.bfloat16)


def _permute_wo(wo_ref, out_ref):
    ntiles, D = wo_ref.shape[0], out_ref.shape[0]
    half = D // _A_HEADS // 2
    for t in range(ntiles):
        w32 = wo_ref.at[t].bitcast(jnp.uint32)
        for i in range(half):
            for k, rows in enumerate(_unpack_rows(w32[pl.ds(i, _A_HEADS, stride=half), :])):
                out_ref[pl.ds((2 * i + k) * _A_HEADS, _A_HEADS), pl.ds(t * 128, 128)] = rows


def _unpack_rows(w32):
    even = pltpu.bitcast(w32 << 16, jnp.float32).astype(jnp.bfloat16)
    odd = pltpu.bitcast(w32 & jnp.uint32(0xFFFF0000), jnp.float32).astype(jnp.bfloat16)
    return even, odd


def _project_a(j, r0, ax_ref, wqkv_ref, scr):
    D = ax_ref.shape[1]
    y = _dot(ax_ref[pl.ds(r0, _RP), :], wqkv_ref[:, j * D:(j + 1) * D])
    if j == 0:
        scr[pl.ds(r0, _RP), :] = y * ((D // _A_HEADS) ** -0.5 * _LOG2E)
    else:
        for n in range(_NSHIFT):
            scr.at[n, pl.ds(r0, _RP + 2 * _HALO), :][pl.ds(_HALO + n * _A_DIL, _RP), :] = y


def _attend_a(r0, q_scr, k_scr, v_scr):
    D = q_scr.shape[1]
    for c in range(0, _RO, _CA):
        n = min(_CA, _RO - c)
        c0 = r0 + c
        rows = pl.ds(pl.multiple_of(c0, 8), n)
        q = q_scr[rows, :]
        tap = lambda scr, w: scr[w % _NSHIFT, pl.ds(pl.multiple_of(c0 + (_HALO - w // _NSHIFT * 8), 8), n), :]
        logits = []
        for w in range(_A_WIN):
            prod = q * tap(k_scr, w)
            lg = functools.reduce(jnp.add, [prod[:, t:t + 128] for t in range(0, D, 128)])
            lg = lg + pltpu.roll(lg, 2 * _A_HEADS, 1)
            lg = lg + pltpu.roll(lg, _A_HEADS, 1)
            if c < w * _A_DIL:
                pos = c0 + jax.lax.broadcasted_iota(jnp.int32, lg.shape, 0)
                lg = jnp.where(pos >= w * _A_DIL, lg, _NEG * _LOG2E)
            logits.append(lg)
        m = functools.reduce(jnp.maximum, logits)
        e = [jnp.exp2(lg - m) for lg in logits]
        inv = _recip(functools.reduce(jnp.add, e))
        o = None
        for w in range(_A_WIN):
            t = jnp.concatenate([e[w]] * (D // 128), axis=1) * tap(v_scr, w)
            o = t if o is None else o + t
        q_scr[rows, :] = o * jnp.concatenate([inv] * (D // 128), axis=1)


def _head_pair(w32):
    return jnp.concatenate(_unpack_rows(w32), axis=1)


def _project(slot, rows, which, bx_ref, c_ref, wq_ref, wuk_ref, wuv_ref, q_scr, k_scr, v_scr):
    if which == 0:
        d = wq_ref.shape[2]
        q = _dot(bx_ref[rows, :], _head_pair(wq_ref[slot])) * (d ** -0.5 * _LOG2E)
        q_scr[slot, rows, :] = q.astype(jnp.bfloat16)
    else:
        c = c_ref[rows, :]
        k_scr[slot, :, rows] = _dot(c, _head_pair(wuk_ref[slot])).T.astype(jnp.bfloat16)
        v_scr[slot, rows, :] = _dot(c, _head_pair(wuv_ref[slot])).astype(jnp.bfloat16)


def _attend(pair, slot, hh, i, q_scr, k_scr, v_scr, ctx_scr):
    d = q_scr.shape[2] // 2
    hs = slice(hh * d, (hh + 1) * d)
    lo, hi = i * _BQ, (i + 1) * _BQ
    nsub = _BQ // _SB
    row = jax.lax.broadcasted_iota(jnp.int32, (_SB, _SB), 0)
    col = jax.lax.broadcasted_iota(jnp.int32, (_SB, _SB), 1)
    sub = lambda x, j: x[j * _SB:(j + 1) * _SB]
    q = q_scr[slot, lo:hi, hs]
    spans = ([(0, lo, 0)] if i > 0 else []) + [(lo + t * _SB, lo + (t + 1) * _SB, t) for t in range(nsub)]
    s = {}
    for n, (k0, k1, t) in enumerate(spans):
        sn = _dot(q[t * _SB:], k_scr[slot, hs, k0:k1])
        for j in range(t, nsub):
            sj = sub(sn, j - t)
            s[n, j] = jnp.where(col <= row, sj, _NEG * _LOG2E) if (k0 >= lo and j == t) else sj
    p, inv = {}, []
    for j in range(nsub):
        keys = [key for key in s if key[1] == j]
        tiles = [s[key][:, c:c + 128] for key in keys for c in range(0, s[key].shape[1], 128)]
        m = jnp.max(functools.reduce(jnp.maximum, tiles), axis=-1, keepdims=True)
        l = None
        for key in keys:
            cols = []
            for c in range(0, s[key].shape[1], 128):
                e = jnp.exp2(s[key][:, c:c + 128] - m)
                l = e if l is None else l + e
                cols.append(e.astype(jnp.bfloat16))
            p[key] = jnp.concatenate(cols, axis=1)
        inv.append(_recip(jnp.sum(l, axis=-1, keepdims=True)))
    ctx = [None] * nsub
    for n, (k0, k1, t) in enumerate(spans):
        pn = jnp.concatenate([p[n, j] for j in range(t, nsub)], axis=0)
        cn = _dot(pn, v_scr[slot, k0:k1, hs])
        for j in range(t, nsub):
            ctx[j] = sub(cn, j - t) if ctx[j] is None else ctx[j] + sub(cn, j - t)
    for j in range(nsub):
        ctx_scr[pair, lo + j * _SB:lo + (j + 1) * _SB, hs] = (ctx[j] * inv[j]).astype(jnp.bfloat16)


def _kernel(ax_hbm, wqkv_hbm, wo_hbm, bx_hbm, c_hbm, wq_hbm, wuk_hbm, wuv_hbm, wob_hbm, o_hbm,
            ax, wqkv, wo_raw, bx, c, wob, wo, wq2, wuk2, wuv2,
            qa_scr, ka_scr, va_scr, q_scr, k_scr, v_scr, ctx_scr, in_sem, ax_sem, wa_sem, wo_sem, w_sem, ob_sem):
    S, DA = ax.shape
    M = bx.shape[1]
    npairs = ctx_scr.shape[0]
    srcs = (bx_hbm, c_hbm, wob_hbm)
    dsts = (bx, c, wob)
    loads = [pltpu.make_async_copy(s, t, in_sem.at[n]) for n, (s, t) in enumerate(zip(srcs, dsts))]

    wo_loads = [pltpu.make_async_copy(wo_hbm.at[:, pl.ds(t * 128, 128)], wo_raw.at[t, pl.ds(0, DA), :], wo_sem.at[t])
                for t in range(DA // 128)]

    def pair_loads(pair):
        return [pltpu.make_async_copy(w.bitcast(jnp.uint32).at[:, pair, :], t.at[pair % 2], w_sem.at[n, pair % 2])
                for n, (w, t) in enumerate(((wq_hbm, wq2), (wuk_hbm, wuk2), (wuv_hbm, wuv2)))]

    wqkv_loads = [pltpu.make_async_copy(wqkv_hbm.at[:, pl.ds(j * DA, DA)], wqkv.at[:, pl.ds(j * DA, DA)],
                                        wa_sem.at[j]) for j in range(3)]
    nblk = S // _RP

    def ax_load(blk):
        rows = pl.ds(blk * _RP, _RP)
        return pltpu.make_async_copy(ax_hbm.at[rows, :], ax.at[rows, :], ax_sem.at[blk])

    for cp in [wqkv_loads[0], ax_load(0), wqkv_loads[1]] + [ax_load(n) for n in range(1, nblk)] + wqkv_loads[2:]:
        cp.start()
    ka_scr[:, 0:2 * _HALO, :] = jnp.zeros((_NSHIFT, 2 * _HALO, DA), jnp.float32)
    va_scr[:, 0:2 * _HALO, :] = jnp.zeros((_NSHIFT, 2 * _HALO, DA), jnp.float32)
    wqkv_loads[0].wait()
    _permute_wqkv(wqkv, 0, pl.ds(0, DA))
    wrows = DA // nblk
    proj = (bx, c, wq2, wuk2, wuv2, q_scr, k_scr, v_scr)
    qkv = (q_scr, k_scr, v_scr, ctx_scr)
    nq = S // _BQ
    for j, scr in enumerate((qa_scr, ka_scr, va_scr)):
        if j < 2:
            wqkv_loads[j + 1].wait()
        else:
            for cp in loads[:2] + pair_loads(0):
                cp.wait()

        @pl.loop(0, nblk)
        def _(blk):
            if j == 0:
                ax_load(blk).wait()

                @pl.when(blk == 0)
                def _():
                    for cp in loads[:2] + pair_loads(0) + wo_loads + pair_loads(1) + loads[2:]:
                        cp.start()

            _project_a(j, pl.multiple_of(blk * _RP, _RP), ax, wqkv, scr)
            if j < 2:
                _permute_wqkv(wqkv, j + 1, pl.ds(pl.multiple_of(blk * wrows, wrows), wrows))
            else:
                for which in range(2):
                    _project(0, pl.ds(pl.multiple_of(blk * _RP, _RP), _RP), which, *proj)

    for cp in wo_loads:
        cp.wait()
    _permute_wo(wo_raw, wo)

    @pl.loop(0, npairs - 1)
    def _(pair):
        slot = pair % 2

        @pl.when(pair + 2 < npairs)
        def _():
            for cp in pair_loads(pair + 2):
                cp.start()

        for cp in pair_loads(pair + 1):
            cp.wait()
        for i in reversed(range(nq)):
            for hh in range(2):
                _attend(pair, slot, hh, i, *qkv)
        for r0 in range(0, S, _PJ):
            for which in range(2):
                _project(1 - slot, pl.ds(r0, _PJ), which, *proj)

    last = npairs - 1
    for i in reversed(range(nq)):
        for hh in range(2):
            _attend(last, last % 2, hh, i, *qkv)

    def stores(i):
        rows = pl.ds(i * _RO, _RO)
        return [pltpu.make_async_copy(ax.at[rows, :], o_hbm.at[rows, pl.ds(0, DA)], ob_sem.at[0, i]),
                pltpu.make_async_copy(bx.at[rows, :], o_hbm.at[rows, pl.ds(DA, M)], ob_sem.at[1, i])]

    loads[2].wait()

    @pl.loop(0, S // _RO)
    def _(i):
        r0 = pl.multiple_of(i * _RO, _RO)
        rows = pl.ds(r0, _RO)
        _attend_a(r0, qa_scr, ka_scr, va_scr)
        ctx = jnp.concatenate([ctx_scr[p, rows, :] for p in range(npairs)], axis=1)
        bx[rows, :] = _dot(ctx, wob[...]).astype(o_hbm.dtype)
        ax[rows, :] = _dot(qa_scr[rows, :].astype(jnp.bfloat16), wo[...]).astype(o_hbm.dtype)
        for cp in stores(i):
            cp.start()

    for i in range(S // _RO):
        for cp in stores(i):
            cp.wait()


@jax.jit
def pallas_concat_heads__sliding_local_dilated__compressed_kv_cla__prompt_kernel(
    A_x: jax.Array,
    A_wqkv: jax.Array,
    A_wo: jax.Array,
    B_x: jax.Array,
    B_c_kv: jax.Array,
    B_w_q: jax.Array,
    B_w_uk: jax.Array,
    B_w_uv: jax.Array,
    B_w_o: jax.Array,
):
    B, S, DA = A_x.shape
    _, _, M = B_x.shape
    _, Sk, Dc = B_c_kv.shape
    _, H, d = B_w_q.shape
    assert DA % 128 == 0 and 4 * _A_HEADS == 128 and B == 1 and Sk == S and H % 2 == 0
    bf16 = jnp.bfloat16
    operands = (A_x.reshape(S, DA), A_wqkv, A_wo, B_x.reshape(S, M), B_c_kv.reshape(Sk, Dc),
                B_w_q, B_w_uk, B_w_uv,
                B_w_o.reshape(H * d, M))
    assert all(a.dtype == bf16 for a in operands)
    hbm = pl.BlockSpec(memory_space=pltpu.HBM)
    out = pl.pallas_call(
        _kernel,
        in_specs=[hbm] * len(operands),
        out_specs=hbm,
        out_shape=jax.ShapeDtypeStruct((S, DA + M), bf16),
        scratch_shapes=[
            pltpu.VMEM((S, DA), bf16),
            pltpu.VMEM((DA, 3 * DA), bf16),
            pltpu.VMEM((DA // 128, DA + 32, 128), bf16),
            pltpu.VMEM((S, M), bf16),
            pltpu.VMEM((Sk, Dc), bf16),
            pltpu.VMEM((H * d, M), bf16),
            pltpu.VMEM((DA, DA), bf16),
            pltpu.VMEM((2, M, d), jnp.uint32),
            pltpu.VMEM((2, Dc, d), jnp.uint32),
            pltpu.VMEM((2, Dc, d), jnp.uint32),
            pltpu.VMEM((S, DA), jnp.float32),
            pltpu.VMEM((_NSHIFT, S + 2 * _HALO, DA), jnp.float32),
            pltpu.VMEM((_NSHIFT, S + 2 * _HALO, DA), jnp.float32),
            pltpu.VMEM((2, S, 2 * d), bf16),
            pltpu.VMEM((2, 2 * d, S), bf16),
            pltpu.VMEM((2, S, 2 * d), bf16),
            pltpu.VMEM((H // 2, S, 2 * d), bf16),
            pltpu.SemaphoreType.DMA((3,)),
            pltpu.SemaphoreType.DMA((S // _RP,)),
            pltpu.SemaphoreType.DMA((3,)),
            pltpu.SemaphoreType.DMA((DA // 128,)),
            pltpu.SemaphoreType.DMA((3, 2)),
            pltpu.SemaphoreType.DMA((2, S // _RO)),
        ],
        compiler_params=pltpu.CompilerParams(vmem_limit_bytes=120 * 1024 * 1024),
    )(*operands)
    return out.reshape(B, S, DA + M)
```

```python
import functools

import jax
import jax.numpy as jnp
import jax.experimental.pallas as pl
import jax.experimental.pallas.tpu as pltpu

_LOG2E = 1.4426950408889634
_NEG = -1e9

_A_HEADS = 32
_A_WIN = 8
_A_DIL = 2
_NSHIFT = 8 // _A_DIL
_HALO = 8

_BQ = 512
_SB = 128
_CA = 16
_RP = 512
_RO = 256
_PJ = 1024


def _dot(a, b):
    return jnp.dot(a, b, preferred_element_type=jnp.float32)


def _recip(x):
    r = pl.reciprocal(x, approx=True)
    return r * (2.0 - x * r)


def _permute_wqkv(wqkv_ref, j, rows):
    D = wqkv_ref.shape[0]
    dh = D // _A_HEADS
    tiles = [pltpu.bitcast(wqkv_ref[rows, pl.ds(j * D + t, 128)], jnp.uint32) for t in range(0, D, 128)]
    lane = jax.lax.broadcasted_iota(jnp.int32, tiles[0].shape, 1)
    for t in range(0, D, 128):
        src = (lane % _A_HEADS) * dh + (lane + t) // _A_HEADS
        out = None
        for n, tile in enumerate(tiles):
            g = jnp.take_along_axis(tile, src % 128, axis=1)
            out = g if out is None else jnp.where(src // 128 == n, g, out)
        wqkv_ref[rows, pl.ds(j * D + t, 128)] = pltpu.bitcast(out, jnp.bfloat16)


def _permute_wo(wo_ref, out_ref):
    ntiles, D = wo_ref.shape[0], out_ref.shape[0]
    half = D // _A_HEADS // 2
    for t in range(ntiles):
        w32 = wo_ref.at[t].bitcast(jnp.uint32)
        for i in range(half):
            for k, rows in enumerate(_unpack_rows(w32[pl.ds(i, _A_HEADS, stride=half), :])):
                out_ref[pl.ds((2 * i + k) * _A_HEADS, _A_HEADS), pl.ds(t * 128, 128)] = rows


def _unpack_rows(w32):
    even = pltpu.bitcast(w32 << 16, jnp.float32).astype(jnp.bfloat16)
    odd = pltpu.bitcast(w32 & jnp.uint32(0xFFFF0000), jnp.float32).astype(jnp.bfloat16)
    return even, odd


def _project_a(j, r0, ax_ref, wqkv_ref, scr):
    D = ax_ref.shape[1]
    y = _dot(ax_ref[pl.ds(r0, _RP), :], wqkv_ref[:, j * D:(j + 1) * D])
    if j == 0:
        scr[pl.ds(r0, _RP), :] = y * ((D // _A_HEADS) ** -0.5 * _LOG2E)
    else:
        for n in range(_NSHIFT):
            scr.at[n, pl.ds(r0, _RP + 2 * _HALO), :][pl.ds(_HALO + n * _A_DIL, _RP), :] = y


def _attend_a(r0, q_scr, k_scr, v_scr):
    D = q_scr.shape[1]
    for c in range(0, _RO, _CA):
        n = min(_CA, _RO - c)
        c0 = r0 + c
        rows = pl.ds(pl.multiple_of(c0, 8), n)
        q = q_scr[rows, :]
        tap = lambda scr, w: scr[w % _NSHIFT, pl.ds(pl.multiple_of(c0 + (_HALO - w // _NSHIFT * 8), 8), n), :]
        logits = []
        for w in range(_A_WIN):
            prod = q * tap(k_scr, w)
            lg = functools.reduce(jnp.add, [prod[:, t:t + 128] for t in range(0, D, 128)])
            lg = lg + pltpu.roll(lg, 2 * _A_HEADS, 1)
            lg = lg + pltpu.roll(lg, _A_HEADS, 1)
            if c < w * _A_DIL:
                pos = c0 + jax.lax.broadcasted_iota(jnp.int32, lg.shape, 0)
                lg = jnp.where(pos >= w * _A_DIL, lg, _NEG * _LOG2E)
            logits.append(lg)
        m = functools.reduce(jnp.maximum, logits)
        e = [jnp.exp2(lg - m) for lg in logits]
        inv = _recip(functools.reduce(jnp.add, e))
        o = None
        for w in range(_A_WIN):
            t = jnp.concatenate([e[w]] * (D // 128), axis=1) * tap(v_scr, w)
            o = t if o is None else o + t
        q_scr[rows, :] = o * jnp.concatenate([inv] * (D // 128), axis=1)


def _head_pair(w32):
    return jnp.concatenate(_unpack_rows(w32), axis=1)


def _project(slot, rows, which, bx_ref, c_ref, wq_ref, wuk_ref, wuv_ref, q_scr, k_scr, v_scr):
    if which == 0:
        d = wq_ref.shape[2]
        q = _dot(bx_ref[rows, :], _head_pair(wq_ref[slot])) * (d ** -0.5 * _LOG2E)
        q_scr[slot, rows, :] = q.astype(jnp.bfloat16)
    else:
        c = c_ref[rows, :]
        k_scr[slot, :, rows] = _dot(c, _head_pair(wuk_ref[slot])).T.astype(jnp.bfloat16)
        v_scr[slot, rows, :] = _dot(c, _head_pair(wuv_ref[slot])).astype(jnp.bfloat16)


def _attend(pair, slot, hh, i, q_scr, k_scr, v_scr, ctx_scr):
    d = q_scr.shape[2] // 2
    hs = slice(hh * d, (hh + 1) * d)
    lo, hi = i * _BQ, (i + 1) * _BQ
    nsub = _BQ // _SB
    row = jax.lax.broadcasted_iota(jnp.int32, (_SB, _SB), 0)
    col = jax.lax.broadcasted_iota(jnp.int32, (_SB, _SB), 1)
    sub = lambda x, j: x[j * _SB:(j + 1) * _SB]
    q = q_scr[slot, lo:hi, hs]
    spans = ([(0, lo, 0)] if i > 0 else []) + [(lo + t * _SB, lo + (t + 1) * _SB, t) for t in range(nsub)]
    s = {}
    for n, (k0, k1, t) in enumerate(spans):
        sn = _dot(q[t * _SB:], k_scr[slot, hs, k0:k1])
        for j in range(t, nsub):
            sj = sub(sn, j - t)
            s[n, j] = jnp.where(col <= row, sj, _NEG * _LOG2E) if (k0 >= lo and j == t) else sj
    p, inv = {}, []
    for j in range(nsub):
        keys = [key for key in s if key[1] == j]
        tiles = [s[key][:, c:c + 128] for key in keys for c in range(0, s[key].shape[1], 128)]
        m = jnp.max(functools.reduce(jnp.maximum, tiles), axis=-1, keepdims=True)
        l = None
        for key in keys:
            cols = []
            for c in range(0, s[key].shape[1], 128):
                e = jnp.exp2(s[key][:, c:c + 128] - m)
                l = e if l is None else l + e
                cols.append(e.astype(jnp.bfloat16))
            p[key] = jnp.concatenate(cols, axis=1)
        inv.append(_recip(jnp.sum(l, axis=-1, keepdims=True)))
    ctx = [None] * nsub
    for n, (k0, k1, t) in enumerate(spans):
        pn = jnp.concatenate([p[n, j] for j in range(t, nsub)], axis=0)
        cn = _dot(pn, v_scr[slot, k0:k1, hs])
        for j in range(t, nsub):
            ctx[j] = sub(cn, j - t) if ctx[j] is None else ctx[j] + sub(cn, j - t)
    for j in range(nsub):
        ctx_scr[pair, lo + j * _SB:lo + (j + 1) * _SB, hs] = (ctx[j] * inv[j]).astype(jnp.bfloat16)


def _kernel(ax_hbm, wqkv_hbm, wo_hbm, bx_hbm, c_hbm, wq_hbm, wuk_hbm, wuv_hbm, wob_hbm, o_hbm,
            ax, wqkv, wo_raw, bx, c, wob, wo, ob, wq2, wuk2, wuv2,
            qa_scr, ka_scr, va_scr, q_scr, k_scr, v_scr, ctx_scr, in_sem, ax_sem, wa_sem, wo_sem, w_sem, ob_sem):
    S, DA = ax.shape
    M = bx.shape[1]
    npairs = ctx_scr.shape[0]
    srcs = (bx_hbm, c_hbm, wob_hbm)
    dsts = (bx, c, wob)
    loads = [pltpu.make_async_copy(s, t, in_sem.at[n]) for n, (s, t) in enumerate(zip(srcs, dsts))]

    wo_loads = [pltpu.make_async_copy(wo_hbm.at[:, pl.ds(t * 128, 128)], wo_raw.at[t, pl.ds(0, DA), :], wo_sem.at[t])
                for t in range(DA // 128)]

    def pair_loads(pair, slot):
        return [pltpu.make_async_copy(w.bitcast(jnp.uint32).at[:, pair, :], t.at[slot], w_sem.at[n, slot])
                for n, (w, t) in enumerate(((wq_hbm, wq2), (wuk_hbm, wuk2), (wuv_hbm, wuv2)))]

    wqkv_loads = [pltpu.make_async_copy(wqkv_hbm.at[:, pl.ds(j * DA, DA)], wqkv.at[:, pl.ds(j * DA, DA)],
                                        wa_sem.at[j]) for j in range(3)]
    nblk = S // _RP

    def ax_load(blk):
        rows = pl.ds(blk * _RP, _RP)
        return pltpu.make_async_copy(ax_hbm.at[rows, :], ax.at[rows, :], ax_sem.at[blk])

    for cp in [wqkv_loads[0], ax_load(0), wqkv_loads[1]] + [ax_load(n) for n in range(1, nblk)] + wqkv_loads[2:]:
        cp.start()
    ka_scr[:, 0:2 * _HALO, :] = jnp.zeros((_NSHIFT, 2 * _HALO, DA), jnp.float32)
    va_scr[:, 0:2 * _HALO, :] = jnp.zeros((_NSHIFT, 2 * _HALO, DA), jnp.float32)
    wo_raw[:, DA:, :] = jnp.zeros((wo_raw.shape[0], wo_raw.shape[1] - DA, 128), wo_raw.dtype)
    wqkv_loads[0].wait()
    _permute_wqkv(wqkv, 0, pl.ds(0, DA))
    wrows = DA // nblk
    proj = (bx, c, wq2, wuk2, wuv2, q_scr, k_scr, v_scr)
    qkv = (q_scr, k_scr, v_scr, ctx_scr)
    nq = S // _BQ
    for j, scr in enumerate((qa_scr, ka_scr, va_scr)):
        if j < 2:
            wqkv_loads[j + 1].wait()
        else:
            for cp in loads[:2] + pair_loads(0, 0):
                cp.wait()

        @pl.loop(0, nblk)
        def _(blk):
            if j == 0:
                ax_load(blk).wait()

                @pl.when(blk == 0)
                def _():
                    for cp in loads[:2] + pair_loads(0, 0) + wo_loads + pair_loads(1, 1) + loads[2:]:
                        cp.start()

            _project_a(j, pl.multiple_of(blk * _RP, _RP), ax, wqkv, scr)
            if j < 2:
                _permute_wqkv(wqkv, j + 1, pl.ds(pl.multiple_of(blk * wrows, wrows), wrows))
            else:
                for which in range(2):
                    _project(0, pl.ds(pl.multiple_of(blk * _RP, _RP), _RP), which, *proj)

    @pl.loop(0, npairs - 1)
    def _(pair):
        slot = pair % 2

        for cp in pair_loads(jnp.minimum(pair + 2, npairs - 1), slot):
            cp.start()
        for cp in pair_loads(pair + 1, 1 - slot):
            cp.wait()
        for i in reversed(range(nq)):
            for hh in range(2):
                _attend(pair, slot, hh, i, *qkv)
        for r0 in range(0, S, _PJ):
            for which in range(2):
                _project(1 - slot, pl.ds(r0, _PJ), which, *proj)

    for cp in pair_loads(npairs - 1, npairs % 2) + wo_loads:
        cp.wait()
    _permute_wo(wo_raw, wo)
    last = npairs - 1
    for i in reversed(range(nq)):
        for hh in range(2):
            _attend(last, last % 2, hh, i, *qkv)

    def stores(i):
        rows = pl.ds(i * _RO, _RO)
        return [pltpu.make_async_copy(ax.at[rows, :], o_hbm.at[rows, pl.ds(0, DA)], ob_sem.at[0, i]),
                pltpu.make_async_copy(ob.at[rows, :], o_hbm.at[rows, pl.ds(DA, M)], ob_sem.at[1, i])]

    loads[2].wait()

    @pl.loop(0, S // _RO)
    def _(i):
        r0 = pl.multiple_of(i * _RO, _RO)
        rows = pl.ds(r0, _RO)
        _attend_a(r0, qa_scr, ka_scr, va_scr)
        ctx = jnp.concatenate([ctx_scr[p, rows, :] for p in range(npairs)], axis=1)
        ob[rows, :] = _dot(ctx, wob[...]).astype(o_hbm.dtype)
        ax[rows, :] = _dot(qa_scr[rows, :].astype(jnp.bfloat16), wo[...]).astype(o_hbm.dtype)
        for cp in stores(i):
            cp.start()

    for i in range(S // _RO):
        for cp in stores(i):
            cp.wait()


@jax.jit
def pallas_concat_heads__sliding_local_dilated__compressed_kv_cla__prompt_kernel(
    A_x: jax.Array,
    A_wqkv: jax.Array,
    A_wo: jax.Array,
    B_x: jax.Array,
    B_c_kv: jax.Array,
    B_w_q: jax.Array,
    B_w_uk: jax.Array,
    B_w_uv: jax.Array,
    B_w_o: jax.Array,
):
    B, S, DA = A_x.shape
    _, _, M = B_x.shape
    _, Sk, Dc = B_c_kv.shape
    _, H, d = B_w_q.shape
    assert DA % 128 == 0 and 4 * _A_HEADS == 128 and B == 1 and Sk == S and H % 2 == 0
    bf16 = jnp.bfloat16
    operands = (A_x.reshape(S, DA), A_wqkv, A_wo, B_x.reshape(S, M), B_c_kv.reshape(Sk, Dc),
                B_w_q, B_w_uk, B_w_uv,
                B_w_o.reshape(H * d, M))
    assert all(a.dtype == bf16 for a in operands)
    hbm = pl.BlockSpec(memory_space=pltpu.HBM)
    out = pl.pallas_call(
        _kernel,
        in_specs=[hbm] * len(operands),
        out_specs=hbm,
        out_shape=jax.ShapeDtypeStruct((S, DA + M), bf16),
        scratch_shapes=[
            pltpu.VMEM((S, DA), bf16),
            pltpu.VMEM((DA, 3 * DA), bf16),
            pltpu.VMEM((DA // 128, DA + 64, 128), bf16),
            pltpu.VMEM((S, M), bf16),
            pltpu.VMEM((Sk, Dc), bf16),
            pltpu.VMEM((H * d, M), bf16),
            pltpu.VMEM((DA, DA), bf16),
            pltpu.VMEM((S, M), bf16),
            pltpu.VMEM((2, M, d), jnp.uint32),
            pltpu.VMEM((2, Dc, d), jnp.uint32),
            pltpu.VMEM((2, Dc, d), jnp.uint32),
            pltpu.VMEM((S, DA), jnp.float32),
            pltpu.VMEM((_NSHIFT, S + 2 * _HALO, DA), jnp.float32),
            pltpu.VMEM((_NSHIFT, S + 2 * _HALO, DA), jnp.float32),
            pltpu.VMEM((2, S, 2 * d), bf16),
            pltpu.VMEM((2, 2 * d, S), bf16),
            pltpu.VMEM((2, S, 2 * d), bf16),
            pltpu.VMEM((H // 2, S, 2 * d), bf16),
            pltpu.SemaphoreType.DMA((3,)),
            pltpu.SemaphoreType.DMA((S // _RP,)),
            pltpu.SemaphoreType.DMA((3,)),
            pltpu.SemaphoreType.DMA((DA // 128,)),
            pltpu.SemaphoreType.DMA((3, 2)),
            pltpu.SemaphoreType.DMA((2, S // _RO)),
        ],
        compiler_params=pltpu.CompilerParams(vmem_limit_bytes=120 * 1024 * 1024),
    )(*operands)
    return out.reshape(B, S, DA + M)
```
